```python
import jax
import jax.numpy as jnp

def _softmax(x, axis=-1):
    return jax.nn.softmax(x, axis=axis)
def _gelu(x):
    return jax.nn.gelu(x, approximate=True)
def _silu(x):
    return jax.nn.silu(x)
def _sigmoid(x):
    return jax.nn.sigmoid(x)
def _layernorm(x, axis=-1, eps=1e-5):
    m = jnp.mean(x, axis=axis, keepdims=True)
    v = jnp.var(x, axis=axis, keepdims=True)
    return (x - m) / jnp.sqrt(v + eps)
def _scatter_add(tgt, idx, src, axis=0):
    return tgt.at[idx].add(src)
def _segment_sum(src, seg, n):
    return jax.ops.segment_sum(src, seg, n)
class _Rng:
    def __init__(self, key):
        self._k = key
    def _next(self):
        self._k, sub = jax.random.split(self._k)
        return sub
    def normal(self, shape):
        return jax.random.normal(self._next(), shape, dtype=jnp.bfloat16)
    def randint(self, lo, hi, shape):
        return jax.random.randint(self._next(), shape, lo, hi, dtype=jnp.int32)
    def uniform(self, shape, lo=0.0, hi=1.0):
        return jax.random.uniform(self._next(), shape, jnp.bfloat16, lo, hi)
    def permutation(self, n):
        return jax.random.permutation(self._next(), n)


kernel_name = 'standalone__qk_norm__prompt'

def setup_inputs():
    _rng = _Rng(jax.random.key(int.from_bytes(__import__("os").urandom(4), "little")))
    _w = (lambda a: (lambda t: t.astype(jnp.bfloat16) if jnp.issubdtype(t.dtype, jnp.floating) else t)(jnp.asarray(a)))
    B, H, S, D = 2, 32, 2048, 1024
    Dh = D // H
    return {
        "q": _w((lambda *s: _rng.normal(s) * 0.05)(B, H, S, Dh)),
        "k": _w((lambda *s: _rng.normal(s) * 0.05)(B, H, S, Dh)),
        "v": _w((lambda *s: _rng.normal(s) * 0.05)(B, H, S, Dh)),
        "t": _w(jnp.abs((lambda *s: _rng.normal(s) * 0.05)(H)) + 1.0),
    }

def reference(q, k, v, t):
    eps = 1e-6
    qn = q / (jnp.sqrt((q * q).sum(axis=-1, keepdims=True)) + eps)
    kn = k / (jnp.sqrt((k * k).sum(axis=-1, keepdims=True)) + eps)
    logits = jnp.einsum('bhqd,bhkd->bhqk', qn, kn) * t[None, :, None, None]
    attn = _softmax(logits, axis=-1)
    return jnp.einsum('bhqk,bhkd->bhqd', attn, v)
```

```python
import functools, math
import jax, jax.numpy as jnp, numpy as np
from jax import lax
from jax.experimental import pallas as pl
from jax.experimental.pallas import tpu as pltpu

LOG2E = 1.4426950408889634
EPS = 1e-6

def make(BQ=256, BK=256, flags=None, qk_first=True, npos=0, NB=128):
    def kernel(t_ref, q_hbm, k_hbm, v_hbm, o_hbm,
               qbuf, kbuf, vbuf, obuf, kn0, kn1, qn0, qn1, s0, s1, m0, m1, sem, *, NH, H, S, D):
        nq, nk = S // BQ, S // BK
        kn = (kn0, kn1); qn = (qn0, qn1); sb = (s0, s1); mb = (m0, m1)

        def cp_q(head, slot): return pltpu.make_async_copy(q_hbm.at[head], qbuf.at[slot], sem.at[0, slot])
        def cp_k(head, slot): return pltpu.make_async_copy(k_hbm.at[head], kbuf.at[slot], sem.at[1, slot])
        def cp_v(head, slot): return pltpu.make_async_copy(v_hbm.at[head], vbuf.at[slot], sem.at[2, slot])
        def cp_o(head, slot): return pltpu.make_async_copy(obuf.at[slot], o_hbm.at[head], sem.at[3, slot])

        def norm_k(p, i):
            x = kbuf[p, :, i * NB:(i + 1) * NB].astype(jnp.float32)
            inv = 1.0 / (jnp.sqrt(jnp.sum(x * x, axis=0, keepdims=True)) + EPS)
            kn[p][i * NB:(i + 1) * NB, :] = (x * inv).T.astype(jnp.bfloat16)

        def norm_q(p, i, scale):
            x = qbuf[p, :, i * NB:(i + 1) * NB].astype(jnp.float32)
            inv = scale / (jnp.sqrt(jnp.sum(x * x, axis=0, keepdims=True)) + EPS)
            qn[p][:, i * NB:(i + 1) * NB] = (x * inv).astype(jnp.bfloat16)

        def qk(p, w, c, m):
            s = jnp.dot(kn[p][c * BK:(c + 1) * BK, :], qn[p][:, w * BQ:(w + 1) * BQ],
                        preferred_element_type=jnp.float32)
            sb[p][c * BK:(c + 1) * BK, w * BQ:(w + 1) * BQ] = s
            mc = jnp.max(s.reshape(BK // 8, 8, BQ), axis=0)
            return mc if m is None else jnp.maximum(m, mc)

        def pv(p, vs, w, c, mrow, l, acc):
            s = sb[p][c * BK:(c + 1) * BK, w * BQ:(w + 1) * BQ]
            pp = jnp.exp2(s - mrow)
            lc = jnp.sum(pp.reshape(BK // 8, 8, BQ), axis=0)
            o = jnp.dot(vbuf[vs, :, c * BK:(c + 1) * BK], pp.astype(jnp.bfloat16),
                        preferred_element_type=jnp.float32)
            return (lc if l is None else l + lc), (o if acc is None else acc + o)

        def stage(j, p, do_n, do_qk, do_pv):
            npieces = 2 * S // NB
            nsteps = nq * nk
            if do_n:
                scale = t_ref[jnp.minimum(j, NH - 1) % H] * LOG2E
            done = 0
            for w in range(nq):
                m = l = acc = None
                if do_pv:
                    mrow = mb[p][:, w * BQ:(w + 1) * BQ]
                for c in range(nk):
                    if qk_first and do_qk: m = qk(1 - p, w, c, m)
                    if do_pv: l, acc = pv(p, p, w, c, mrow, l, acc)
                    if not qk_first and do_qk: m = qk(1 - p, w, c, m)
                    if do_n:
                        step = w * nk + c + 1
                        while done < npieces and done * nsteps < step * npieces:
                            if done % 2 == 0: norm_k(p, done // 2)
                            else: norm_q(p, done // 2, scale)
                            done += 1
                if do_pv:
                    lrow = jnp.sum(l, axis=0, keepdims=True)
                    obuf[p, :, w * BQ:(w + 1) * BQ] = (acc * (1.0 / lrow)).astype(obuf.dtype)
                if do_qk:
                    mb[1 - p][:, w * BQ:(w + 1) * BQ] = jnp.max(m, axis=0, keepdims=True)

        cp_q(0, 0).start(); cp_k(0, 0).start()
        cp_q(1, 1).start(); cp_k(1, 1).start()
        cp_v(0, 0).start()
        cp_q(0, 0).wait(); cp_k(0, 0).wait()
        stage(0, 0, True, False, False)
        cp_q(2, 0).start(); cp_k(2, 0).start()
        cp_q(1, 1).wait(); cp_k(1, 1).wait()
        stage(1, 1, True, True, False)

        def body(j, carry):
            for p in range(2):
                @pl.when(j % 2 == p)
                def _(p=p):
                    @pl.when(j + 1 < NH)
                    def _():
                        cp_q(j + 1, 1 - p).start(); cp_k(j + 1, 1 - p).start()
                    cp_v(j - 1, 1 - p).start()
                    @pl.when(j >= 3)
                    def _():
                        cp_o(j - 3, 1 - p).start()
                    @pl.when(j >= 4)
                    def _():
                        cp_o(j - 4, p).wait()
                    @pl.when(j < NH)
                    def _():
                        cp_q(j, p).wait(); cp_k(j, p).wait()
                    cp_v(j - 2, p).wait()
                    stage(j, p, True, True, True)
            return carry
        lax.fori_loop(2, NH + 1, body, 0)

        p = (NH + 1) % 2
        cp_o(NH - 2, 1 - p).start()
        cp_o(NH - 3, p).wait()
        cp_v(NH - 1, p).wait()
        stage(NH + 1, p, False, False, True)
        cp_o(NH - 1, p).start()
        cp_o(NH - 2, 1 - p).wait()
        cp_o(NH - 1, p).wait()

    @jax.jit
    def f(q, k, v, t):
        B, H, S, D = q.shape
        NH = B * H
        qT = jnp.swapaxes(q, 2, 3).reshape(NH, D, S)
        kT = jnp.swapaxes(k, 2, 3).reshape(NH, D, S)
        vT = jnp.swapaxes(v, 2, 3).reshape(NH, D, S)
        any_spec = pl.BlockSpec(memory_space=pl.ANY)
        oT = pl.pallas_call(
            functools.partial(kernel, NH=NH, H=H, S=S, D=D),
            in_specs=[pl.BlockSpec(memory_space=pltpu.SMEM), any_spec, any_spec, any_spec],
            out_specs=any_spec,
            out_shape=jax.ShapeDtypeStruct((NH, D, S), q.dtype),
            scratch_shapes=[pltpu.VMEM((2, D, S), jnp.bfloat16)] * 4
                           + [pltpu.VMEM((S, D), jnp.bfloat16)] * 2
                           + [pltpu.VMEM((D, S), jnp.bfloat16)] * 2
                           + [pltpu.VMEM((S, S), jnp.float32)] * 2
                           + [pltpu.VMEM((1, S), jnp.float32)] * 2
                           + [pltpu.SemaphoreType.DMA((4, 2))],
            compiler_params=pltpu.CompilerParams(
                vmem_limit_bytes=100 * 1024 * 1024,
                **({"flags": flags} if flags else {})),
        )(t.astype(jnp.float32), qT, kT, vT)
        return jnp.swapaxes(oT.reshape(B, H, D, S), 2, 3)
    return f


pallas_standalone__qk_norm__prompt_kernel = make()
```

```python
import functools

import jax
import jax.numpy as jnp
from jax import lax
from jax.experimental import pallas as pl
from jax.experimental.pallas import tpu as pltpu

LOG2E = 1.4426950408889634
EPS = 1e-6

BQ = 256
BK = 128
LEAD = 2
K_SPAN = (0.30, 0.95)
Q_SPAN = (0.10, 0.90)
TAIL_QK, TAIL_PV = 3, 2


def _add_rows(p, acc):
    for r in reversed(range(p.shape[0] // 8)):
        rows = p[r * 8:(r + 1) * 8]
        acc = rows if acc is None else acc + rows
    return acc


def _spread(span, n, total):
    pos = [min(int((span[0] + (span[1] - span[0]) * i / n) * total), total - 1) for i in range(n)]
    assert len(set(pos)) == n
    return pos


def _interleave(qk, n_qk, pv, n_pv, lead):
    dq = dp = 0
    while dq < n_qk or dp < n_pv:
        if dq < n_qk and (dp >= n_pv or (dq - lead) * max(n_pv, 1) <= dp * max(n_qk, 1)):
            next(qk)
            dq += 1
        else:
            next(pv)
            dp += 1


def _attention_kernel(t_hbm, q_hbm, k_hbm, v_hbm, o_hbm,
                      q_buf, k_buf, v_buf, o_buf,
                      kn0, kn1,
                      qn0, qn1,
                      s0, s1,
                      m0, m1,
                      sems, t_vmem, scale_vmem, scale_smem, t_sems,
                      *, n_heads, heads_per_batch, seq, dim):
    nq, nk = seq // BQ, seq // BK
    items = list(range(nq))
    kn, qn, s_buf, m_buf = (kn0, kn1), (qn0, qn1), (s0, s1), (m0, m1)

    def copy_in(src, dst, sem_row):
        return lambda head, slot: pltpu.make_async_copy(src.at[head], dst.at[slot], sems.at[sem_row, slot])

    copy_q, copy_k, copy_v = copy_in(q_hbm, q_buf, 0), copy_in(k_hbm, k_buf, 1), copy_in(v_hbm, v_buf, 2)

    def copy_o(head, slot):
        return pltpu.make_async_copy(o_buf.at[slot], o_hbm.at[head], sems.at[3, slot])

    def scale_of(head):
        return scale_smem[0, jnp.minimum(head, n_heads - 1) % heads_per_batch]

    def inv_norm(x):
        return 1.0 / (jnp.sqrt(jnp.sum(x * x, axis=0, keepdims=True)) + EPS)

    def norm_k(bank, i):
        x = k_buf[bank, :, i * BK:(i + 1) * BK].astype(jnp.float32)
        piece = (x * inv_norm(x)).T.astype(jnp.bfloat16)
        kn[bank][i * BK:(i + 1) * BK, :] = piece
        return piece

    def norm_q(bank, i, scale, pin=None):
        x = q_buf[bank, :, i * BK:(i + 1) * BK].astype(jnp.float32)
        if pin is not None:
            x = jnp.where(pin[0], pin[1], x)
        qn[bank][:, i * BK:(i + 1) * BK] = (x * (scale * inv_norm(x))).astype(jnp.bfloat16)

    def qk_steps(bank, work, pin_at=None):
        for n, w in enumerate(work):
            cols = slice(w * BQ, (w + 1) * BQ)
            m = None
            for c in range(nk):
                rows = slice(c * BK, (c + 1) * BK)
                lhs = kn[bank][rows, :]
                pin = pin_at(n * nk + c) if pin_at else None
                if pin is not None:
                    lhs = jnp.concatenate([jnp.where(pin[0], pin[1], lhs[0:16]), lhs[16:]], axis=0)
                s = jnp.dot(lhs, qn[bank][:, cols], preferred_element_type=jnp.float32)
                s_buf[bank][rows, cols] = s
                chunk_max = jnp.max(s.reshape(BK // 8, 8, BQ), axis=0)
                m = chunk_max if m is None else jnp.maximum(m, chunk_max)
                if c == nk - 1:
                    m_buf[bank][:, cols] = jnp.max(m, axis=0, keepdims=True)
                yield

    def pv_steps(bank, work, on_p=None):
        for n, w in enumerate(work):
            cols = slice(w * BQ, (w + 1) * BQ)
            m = m_buf[bank][:, cols]
            l = acc = None
            for c in range(nk):
                rows = slice(c * BK, (c + 1) * BK)
                p = jnp.exp2(s_buf[bank][rows, cols] - m)
                l = _add_rows(p, l)
                if on_p is not None:
                    on_p(n * nk + c, p)
                o = jnp.dot(v_buf[bank, :, rows], p.astype(jnp.bfloat16), preferred_element_type=jnp.float32)
                acc = o if acc is None else acc + o
                if c == nk - 1:
                    denom = jnp.sum(l, axis=0, keepdims=True)
                    o_buf[bank, :, cols] = (acc * (1.0 / denom)).astype(o_buf.dtype)
                yield

    def run(qk_bank, qk_work, pv_bank, pv_work, pin_k=None, on_p=None):
        _interleave(qk_steps(qk_bank, qk_work, pin_k), len(qk_work) * nk,
                    pv_steps(pv_bank, pv_work, on_p), len(pv_work) * nk, LEAD)

    def stage(j, bank, qk_work, normalise=True):
        if not normalise:
            return run(1 - bank, qk_work, bank, items)
        never = j < 0
        scale = scale_of(j)
        k_at = {step: norm_k(bank, i)[BK - 16:BK] for i, step in enumerate(_spread(K_SPAN, nk, len(qk_work) * nk))}
        q_at = {step: i for i, step in enumerate(_spread(Q_SPAN, nk, nq * nk))}

        def pin_k(step):
            return (never, k_at[step]) if step in k_at else None

        def on_p(step, p):
            if step in q_at:
                norm_q(bank, q_at[step], scale, (never, p[0:dim, 0:BK]))

        run(1 - bank, qk_work, bank, items, pin_k, on_p)

    def normalise_all(head, bank):
        scale = scale_of(head)
        for i in range(nk):
            norm_k(bank, i)
            norm_q(bank, i, scale)

    t_in = pltpu.make_async_copy(t_hbm, t_vmem, t_sems.at[0])
    t_in.start()
    copy_k(0, 0).start()
    copy_q(0, 0).start()
    t_in.wait()
    scale_vmem[...] = t_vmem[...].astype(jnp.float32) * LOG2E
    t_out = pltpu.make_async_copy(scale_vmem, scale_smem, t_sems.at[1])
    t_out.start()
    t_out.wait()
    copy_q(0, 0).wait()
    copy_k(0, 0).wait()
    copy_k(1, 1).start()
    copy_q(1, 1).start()
    copy_v(0, 0).start()
    normalise_all(0, 0)
    copy_q(2, 0).start()
    copy_k(2, 0).start()
    run(0, items[:1], 0, [])
    copy_q(1, 1).wait()
    copy_k(1, 1).wait()
    normalise_all(1, 1)
    run(0, items[1:], 0, [])

    def steady(j, _):
        for bank in range(2):
            @pl.when(j % 2 == bank)
            def _(bank=bank):
                @pl.when(j + 1 < n_heads)
                def _():
                    copy_q(j + 1, 1 - bank).start()
                    copy_k(j + 1, 1 - bank).start()

                copy_v(j - 1, 1 - bank).start()

                @pl.when(j >= 3)
                def _():
                    copy_o(j - 3, 1 - bank).start()

                @pl.when(j >= 4)
                def _():
                    copy_o(j - 4, bank).wait()

                copy_q(j, bank).wait()
                copy_k(j, bank).wait()
                copy_v(j - 2, bank).wait()
                stage(j, bank, items)
        return j

    last = lax.fori_loop(2, n_heads, steady, jnp.int32(1))

    bank = n_heads % 2
    copy_v(n_heads - 1, 1 - bank).start()
    copy_o(n_heads - 3, 1 - bank).start()
    copy_o(n_heads - 4, bank).wait()
    copy_v(n_heads - 2, bank).wait()
    stage(last + 1, bank, items[:nq - TAIL_QK], normalise=False)

    bank = 1 - bank
    copy_o(n_heads - 2, 1 - bank).start()
    copy_o(n_heads - 3, bank).wait()
    copy_v(n_heads - 1, bank).wait()

    @pl.when(last > 0)
    def _():
        run(bank, items[nq - TAIL_QK:], bank, items[:nq - TAIL_PV])

    run(bank, [], bank, items[nq - TAIL_PV:])
    copy_o(n_heads - 1, bank).start()
    copy_o(n_heads - 2, 1 - bank).wait()
    copy_o(n_heads - 1, bank).wait()


def _attention(q, k, v, t, interpret=False):
    batch, heads, seq, dim = q.shape
    n_heads = batch * heads
    assert seq % BQ == 0 and n_heads >= 4 and dim <= BK and seq // BQ > max(TAIL_QK, TAIL_PV)

    def to_head_major(x):
        return jnp.swapaxes(x, 2, 3).reshape(n_heads, dim, seq)

    in_hbm = pl.BlockSpec(memory_space=pl.ANY)
    out = pl.pallas_call(
        functools.partial(_attention_kernel, n_heads=n_heads, heads_per_batch=heads, seq=seq, dim=dim),
        in_specs=[in_hbm] * 4,
        out_specs=in_hbm,
        out_shape=jax.ShapeDtypeStruct((n_heads, dim, seq), q.dtype),
        scratch_shapes=(
            [pltpu.VMEM((2, dim, seq), q.dtype)] * 4
            + [pltpu.VMEM((seq, dim), jnp.bfloat16)] * 2
            + [pltpu.VMEM((dim, seq), jnp.bfloat16)] * 2
            + [pltpu.VMEM((seq, seq), jnp.float32)] * 2
            + [pltpu.VMEM((1, seq), jnp.float32)] * 2
            + [pltpu.SemaphoreType.DMA((4, 2)),
               pltpu.VMEM((1, heads), t.dtype),
               pltpu.VMEM((1, heads), jnp.float32),
               pltpu.SMEM((1, heads), jnp.float32),
               pltpu.SemaphoreType.DMA((2,))]
        ),
        compiler_params=pltpu.CompilerParams(
            vmem_limit_bytes=100 * 1024 * 1024,
            disable_bounds_checks=True,
        ),
        interpret=interpret,
    )(t.reshape(1, heads), to_head_major(q), to_head_major(k), to_head_major(v))
    return jnp.swapaxes(out.reshape(batch, heads, dim, seq), 2, 3)


@jax.jit
def pallas_standalone__qk_norm__prompt_kernel(
    q: jax.Array,
    k: jax.Array,
    v: jax.Array,
    t: jax.Array,
):
    return _attention(q, k, v, t)
```

```python
import functools

import jax
import jax.numpy as jnp
from jax import lax
from jax.experimental import pallas as pl
from jax.experimental.pallas import tpu as pltpu

LOG2E = 1.4426950408889634
EPS = 1e-6

BQ = 256
BK = 128
LEAD = 2
K_SPAN = (0.30, 0.95)
Q_SPAN = (0.10, 0.90)
TAIL_QK, TAIL_PV = 3, 2


def _add_rows(p, acc):
    for r in reversed(range(p.shape[0] // 8)):
        rows = p[r * 8:(r + 1) * 8]
        acc = rows if acc is None else acc + rows
    return acc


def _spread(span, n, total):
    pos = [min(int((span[0] + (span[1] - span[0]) * i / n) * total), total - 1) for i in range(n)]
    assert len(set(pos)) == n
    return pos


def _interleave(qk, n_qk, pv, n_pv, lead):
    dq = dp = 0
    while dq < n_qk or dp < n_pv:
        if dq < n_qk and (dp >= n_pv or (dq - lead) * max(n_pv, 1) <= dp * max(n_qk, 1)):
            next(qk)
            dq += 1
        else:
            next(pv)
            dp += 1


def _attention_kernel(t_hbm, q_hbm, k_hbm, v_hbm, o_hbm,
                      q_buf, k_buf, v_buf, o_buf,
                      kn0, kn1,
                      qn0, qn1,
                      s0, s1,
                      m0, m1,
                      sems, t_vmem, scale_vmem, scale_smem, t_sems,
                      *, n_heads, heads_per_batch, seq, dim):
    nq, nk = seq // BQ, seq // BK
    items = list(range(nq))
    kn, qn, s_buf, m_buf = (kn0, kn1), (qn0, qn1), (s0, s1), (m0, m1)

    def copy_in(src, dst, sem_row):
        return lambda head, slot: pltpu.make_async_copy(src.at[head], dst.at[slot], sems.at[sem_row, slot])

    copy_q, copy_k, copy_v = copy_in(q_hbm, q_buf, 0), copy_in(k_hbm, k_buf, 1), copy_in(v_hbm, v_buf, 2)

    def copy_o(head, slot):
        return pltpu.make_async_copy(o_buf.at[slot], o_hbm.at[head], sems.at[3, slot])

    def scale_of(head):
        return scale_smem[0, jnp.minimum(head, n_heads - 1) % heads_per_batch]

    def inv_norm(x):
        return 1.0 / (jnp.sqrt(jnp.sum(x * x, axis=0, keepdims=True)) + EPS)

    def norm_k(bank, i):
        x = k_buf[bank, :, i * BK:(i + 1) * BK].astype(jnp.float32)
        piece = (x * inv_norm(x)).T.astype(jnp.bfloat16)
        kn[bank][i * BK:(i + 1) * BK, :] = piece
        return piece

    def norm_q(bank, i, scale, pin=None):
        x = q_buf[bank, :, i * BK:(i + 1) * BK].astype(jnp.float32)
        if pin is not None:
            x = jnp.where(pin[0], pin[1], x)
        qn[bank][:, i * BK:(i + 1) * BK] = (x * (scale * inv_norm(x))).astype(jnp.bfloat16)

    def qk_steps(bank, work, pin_at=None):
        for n, w in enumerate(work):
            cols = slice(w * BQ, (w + 1) * BQ)
            m = None
            for c in range(nk):
                rows = slice(c * BK, (c + 1) * BK)
                lhs = kn[bank][rows, :]
                pin = pin_at(n * nk + c) if pin_at else None
                if pin is not None:
                    lhs = jnp.concatenate([jnp.where(pin[0], pin[1], lhs[0:16]), lhs[16:]], axis=0)
                s = jnp.dot(lhs, qn[bank][:, cols], preferred_element_type=jnp.float32)
                s_buf[bank][rows, cols] = s
                chunk_max = jnp.max(s.reshape(BK // 8, 8, BQ), axis=0)
                m = chunk_max if m is None else jnp.maximum(m, chunk_max)
                if c == nk - 1:
                    m_buf[bank][:, cols] = jnp.max(m, axis=0, keepdims=True)
                yield

    def pv_steps(bank, work, on_p=None):
        for n, w in enumerate(work):
            cols = slice(w * BQ, (w + 1) * BQ)
            m = m_buf[bank][:, cols]
            l = acc = None
            for c in range(nk):
                rows = slice(c * BK, (c + 1) * BK)
                p = jnp.exp2(s_buf[bank][rows, cols] - m)
                l = _add_rows(p, l)
                if on_p is not None:
                    on_p(n * nk + c, p)
                o = jnp.dot(v_buf[bank, :, rows], p.astype(jnp.bfloat16), preferred_element_type=jnp.float32)
                acc = o if acc is None else acc + o
                if c == nk - 1:
                    denom = jnp.sum(l, axis=0, keepdims=True)
                    o_buf[bank, :, cols] = (acc * (1.0 / denom)).astype(o_buf.dtype)
                yield

    def run(qk_bank, qk_work, pv_bank, pv_work, pin_k=None, on_p=None):
        _interleave(qk_steps(qk_bank, qk_work, pin_k), len(qk_work) * nk,
                    pv_steps(pv_bank, pv_work, on_p), len(pv_work) * nk, LEAD)

    def stage(j, bank, qk_work, normalise=True):
        if not normalise:
            return run(1 - bank, qk_work, bank, items)
        never = j < 0
        scale = scale_of(j)
        k_at = {step: norm_k(bank, i)[BK - 16:BK] for i, step in enumerate(_spread(K_SPAN, nk, len(qk_work) * nk))}
        q_at = {step: i for i, step in enumerate(_spread(Q_SPAN, nk, nq * nk))}

        def pin_k(step):
            return (never, k_at[step]) if step in k_at else None

        def on_p(step, p):
            if step in q_at:
                norm_q(bank, q_at[step], scale, (never, p[0:dim, 0:BK]))

        run(1 - bank, qk_work, bank, items, pin_k, on_p)

    def normalise_all(head, bank):
        scale = scale_of(head)
        for i in range(nk):
            norm_k(bank, i)
            norm_q(bank, i, scale)

    t_in = pltpu.make_async_copy(t_hbm, t_vmem, t_sems.at[0])
    t_in.start()
    copy_k(0, 0).start()
    copy_q(0, 0).start()
    t_in.wait()
    scale_vmem[...] = t_vmem[...].astype(jnp.float32) * LOG2E
    t_out = pltpu.make_async_copy(scale_vmem, scale_smem, t_sems.at[1])
    t_out.start()
    t_out.wait()
    copy_q(0, 0).wait()
    copy_k(0, 0).wait()
    copy_k(1, 1).start()
    copy_q(1, 1).start()
    copy_v(0, 0).start()
    normalise_all(0, 0)
    copy_q(2, 0).start()
    copy_k(2, 0).start()
    run(0, items[:1], 0, [])
    copy_q(1, 1).wait()
    copy_k(1, 1).wait()
    normalise_all(1, 1)
    run(0, items[1:], 0, [])

    def prefetch(j, bank):
        @pl.when(j + 1 < n_heads)
        def _():
            copy_q(j + 1, 1 - bank).start()
            copy_k(j + 1, 1 - bank).start()

        copy_v(j - 1, 1 - bank).start()

        @pl.when(j >= 3)
        def _():
            copy_o(j - 3, 1 - bank).start()

    prefetch(jnp.int32(2), 0)

    def steady(j, bank):
        @pl.when(j >= 4)
        def _():
            copy_o(j - 4, bank).wait()

        copy_q(j, bank).wait()
        copy_k(j, bank).wait()
        copy_v(j - 2, bank).wait()
        stage(j, bank, items)
        prefetch(j + 1, 1 - bank)

    def steady_pair(i, _):
        j = 2 + 2 * i
        steady(j, 0)
        steady(j + 1, 1)
        return j + 1

    last = lax.fori_loop(0, (n_heads - 2) // 2, steady_pair, jnp.int32(1))

    bank = n_heads % 2
    copy_o(n_heads - 4, bank).wait()
    copy_v(n_heads - 2, bank).wait()
    stage(last + 1, bank, items[:nq - TAIL_QK], normalise=False)

    bank = 1 - bank
    copy_o(n_heads - 2, 1 - bank).start()
    copy_o(n_heads - 3, bank).wait()
    copy_v(n_heads - 1, bank).wait()

    @pl.when(last > 0)
    def _():
        run(bank, items[nq - TAIL_QK:], bank, items[:nq - TAIL_PV])

    run(bank, [], bank, items[nq - TAIL_PV:])
    copy_o(n_heads - 1, bank).start()
    copy_o(n_heads - 2, 1 - bank).wait()
    copy_o(n_heads - 1, bank).wait()


def _attention(q, k, v, t, interpret=False):
    batch, heads, seq, dim = q.shape
    n_heads = batch * heads
    assert seq % BQ == 0 and n_heads >= 4 and n_heads % 2 == 0 and dim <= BK and seq // BQ > max(TAIL_QK, TAIL_PV)

    def to_head_major(x):
        return jnp.swapaxes(x, 2, 3).reshape(n_heads, dim, seq)

    in_hbm = pl.BlockSpec(memory_space=pl.ANY)
    out = pl.pallas_call(
        functools.partial(_attention_kernel, n_heads=n_heads, heads_per_batch=heads, seq=seq, dim=dim),
        in_specs=[in_hbm] * 4,
        out_specs=in_hbm,
        out_shape=jax.ShapeDtypeStruct((n_heads, dim, seq), q.dtype),
        scratch_shapes=(
            [pltpu.VMEM((2, dim, seq), q.dtype)] * 4
            + [pltpu.VMEM((seq, dim), jnp.bfloat16)] * 2
            + [pltpu.VMEM((dim, seq), jnp.bfloat16)] * 2
            + [pltpu.VMEM((seq, seq), jnp.float32)] * 2
            + [pltpu.VMEM((1, seq), jnp.float32)] * 2
            + [pltpu.SemaphoreType.DMA((4, 2)),
               pltpu.VMEM((1, heads), t.dtype),
               pltpu.VMEM((1, heads), jnp.float32),
               pltpu.SMEM((1, heads), jnp.float32),
               pltpu.SemaphoreType.DMA((2,))]
        ),
        compiler_params=pltpu.CompilerParams(
            vmem_limit_bytes=100 * 1024 * 1024,
            disable_bounds_checks=True,
        ),
        interpret=interpret,
    )(t.reshape(1, heads), to_head_major(q), to_head_major(k), to_head_major(v))
    return jnp.swapaxes(out.reshape(batch, heads, dim, seq), 2, 3)


@jax.jit
def pallas_standalone__qk_norm__prompt_kernel(
    q: jax.Array,
    k: jax.Array,
    v: jax.Array,
    t: jax.Array,
):
    return _attention(q, k, v, t)
```

```python
import functools

import jax
import jax.numpy as jnp
from jax import lax
from jax.experimental import pallas as pl
from jax.experimental.pallas import tpu as pltpu

LOG2E = 1.4426950408889634
EPS = 1e-6

BQ = 256
BK = 128
LEAD = 2
K_SPAN = (0.30, 0.95)
Q_SPAN = (0.10, 0.90)
TAIL_QK, TAIL_PV = 3, 2


def _add_rows(p, acc):
    for r in reversed(range(p.shape[0] // 8)):
        rows = p[r * 8:(r + 1) * 8]
        acc = rows if acc is None else acc + rows
    return acc


def _spread(span, n, total):
    pos = [min(int((span[0] + (span[1] - span[0]) * i / n) * total), total - 1) for i in range(n)]
    assert len(set(pos)) == n
    return pos


def _interleave(qk, n_qk, pv, n_pv, lead):
    dq = dp = 0
    while dq < n_qk or dp < n_pv:
        if dq < n_qk and (dp >= n_pv or (dq - lead) * max(n_pv, 1) <= dp * max(n_qk, 1)):
            next(qk)
            dq += 1
        else:
            next(pv)
            dp += 1


def _attention_kernel(t_hbm, q_hbm, k_hbm, v_hbm, o_hbm,
                      in_buf,
                      first_buf,
                      o_buf,
                      kn0, kn1,
                      qn0, qn1,
                      s0, s1,
                      m0, m1,
                      in_sems, first_sems, o_sems, t_vmem, scale_vmem, scale_smem, t_sems,
                      *, n_heads, heads_per_batch, seq, dim):
    nq, nk = seq // BQ, seq // BK
    items = list(range(nq))
    kn, qn, s_buf, m_buf = (kn0, kn1), (qn0, qn1), (s0, s1), (m0, m1)

    Q, K, V = 0, 1, 2

    def start_inputs(j, slot):
        head = jnp.minimum(j, n_heads - 1)
        pltpu.make_async_copy(q_hbm.at[head], in_buf.at[slot, Q], in_sems.at[slot]).start()
        pltpu.make_async_copy(k_hbm.at[head], in_buf.at[slot, K], in_sems.at[slot]).start()
        pltpu.make_async_copy(v_hbm.at[j - 2], in_buf.at[slot, V], in_sems.at[slot]).start()

    def wait_inputs(slot):
        pltpu.make_async_copy(in_buf.at[slot], in_buf.at[slot], in_sems.at[slot]).wait()

    def copy_first(head):
        return [pltpu.make_async_copy(src.at[head], first_buf.at[head, i], first_sems.at[head, i])
                for i, src in ((K, k_hbm), (Q, q_hbm))]

    def copy_o(head, slot):
        return pltpu.make_async_copy(o_buf.at[slot], o_hbm.at[head], o_sems.at[slot])

    def scale_of(head):
        return scale_smem[0, jnp.minimum(head, n_heads - 1) % heads_per_batch]

    def inv_norm(x):
        return 1.0 / (jnp.sqrt(jnp.sum(x * x, axis=0, keepdims=True)) + EPS)

    def norm_k(src, bank, i):
        x = src[:, i * BK:(i + 1) * BK].astype(jnp.float32)
        piece = (x * inv_norm(x)).T.astype(jnp.bfloat16)
        kn[bank][i * BK:(i + 1) * BK, :] = piece
        return piece

    def norm_q(src, bank, i, scale, pin=None):
        x = src[:, i * BK:(i + 1) * BK].astype(jnp.float32)
        if pin is not None:
            x = jnp.where(pin[0], pin[1], x)
        qn[bank][:, i * BK:(i + 1) * BK] = (x * (scale * inv_norm(x))).astype(jnp.bfloat16)

    def qk_steps(bank, work, pin_at=None):
        for n, w in enumerate(work):
            cols = slice(w * BQ, (w + 1) * BQ)
            m = None
            for c in range(nk):
                rows = slice(c * BK, (c + 1) * BK)
                lhs = kn[bank][rows, :]
                pin = pin_at(n * nk + c) if pin_at else None
                if pin is not None:
                    lhs = jnp.concatenate([jnp.where(pin[0], pin[1], lhs[0:16]), lhs[16:]], axis=0)
                s = jnp.dot(lhs, qn[bank][:, cols], preferred_element_type=jnp.float32)
                s_buf[bank][rows, cols] = s
                chunk_max = jnp.max(s.reshape(BK // 8, 8, BQ), axis=0)
                m = chunk_max if m is None else jnp.maximum(m, chunk_max)
                if c == nk - 1:
                    m_buf[bank][:, cols] = jnp.max(m, axis=0, keepdims=True)
                yield

    def pv_steps(bank, work, on_p=None):
        for n, w in enumerate(work):
            cols = slice(w * BQ, (w + 1) * BQ)
            m = m_buf[bank][:, cols]
            l = acc = None
            for c in range(nk):
                rows = slice(c * BK, (c + 1) * BK)
                p = jnp.exp2(s_buf[bank][rows, cols] - m)
                l = _add_rows(p, l)
                if on_p is not None:
                    on_p(n * nk + c, p)
                o = jnp.dot(in_buf[bank, V, :, rows], p.astype(jnp.bfloat16), preferred_element_type=jnp.float32)
                acc = o if acc is None else acc + o
                if c == nk - 1:
                    denom = jnp.sum(l, axis=0, keepdims=True)
                    o_buf[bank, :, cols] = (acc * (1.0 / denom)).astype(o_buf.dtype)
                yield

    def run(qk_bank, qk_work, pv_bank, pv_work, pin_k=None, on_p=None):
        _interleave(qk_steps(qk_bank, qk_work, pin_k), len(qk_work) * nk,
                    pv_steps(pv_bank, pv_work, on_p), len(pv_work) * nk, LEAD)

    def stage(j, bank, qk_work, normalise=True):
        if not normalise:
            return run(1 - bank, qk_work, bank, items)
        never = j < 0
        scale = scale_of(j)
        k_at = {step: norm_k(in_buf.at[bank, K], bank, i)[BK - 16:BK] for i, step in enumerate(_spread(K_SPAN, nk, len(qk_work) * nk))}
        q_at = {step: i for i, step in enumerate(_spread(Q_SPAN, nk, nq * nk))}

        def pin_k(step):
            return (never, k_at[step]) if step in k_at else None

        def on_p(step, p):
            if step in q_at:
                norm_q(in_buf.at[bank, Q], bank, q_at[step], scale, (never, p[0:dim, 0:BK]))

        run(1 - bank, qk_work, bank, items, pin_k, on_p)

    def normalise_all(head, bank):
        scale = scale_of(head)
        for i in range(nk):
            norm_k(first_buf.at[head, K], bank, i)
            norm_q(first_buf.at[head, Q], bank, i, scale)

    t_in = pltpu.make_async_copy(t_hbm, t_vmem, t_sems.at[0])
    t_in.start()
    for c in copy_first(0):
        c.start()
    t_in.wait()
    scale_vmem[...] = t_vmem[...].astype(jnp.float32) * LOG2E
    t_out = pltpu.make_async_copy(scale_vmem, scale_smem, t_sems.at[1])
    t_out.start()
    t_out.wait()
    for c in copy_first(0):
        c.wait()
    for c in copy_first(1):
        c.start()
    start_inputs(2, 0)
    start_inputs(3, 1)
    normalise_all(0, 0)
    run(0, items[:1], 0, [])
    for c in copy_first(1):
        c.wait()
    normalise_all(1, 1)
    run(0, items[1:], 0, [])

    def steady(j, bank):
        @pl.when(j >= 4)
        def _():
            copy_o(j - 4, bank).wait()

        wait_inputs(bank)
        stage(j, bank, items)
        start_inputs(j + 2, bank)
        copy_o(j - 2, bank).start()

    def steady_pair(i, _):
        j = 2 + 2 * i
        steady(j, 0)
        steady(j + 1, 1)
        return j + 1

    last = lax.fori_loop(0, (n_heads - 2) // 2, steady_pair, jnp.int32(1))

    bank = n_heads % 2
    copy_o(n_heads - 4, bank).wait()
    wait_inputs(bank)
    stage(last + 1, bank, items[:nq - TAIL_QK], normalise=False)
    copy_o(n_heads - 2, bank).start()

    bank = 1 - bank
    copy_o(n_heads - 3, bank).wait()
    wait_inputs(bank)

    @pl.when(last > 0)
    def _():
        run(bank, items[nq - TAIL_QK:], bank, items[:nq - TAIL_PV])

    run(bank, [], bank, items[nq - TAIL_PV:])
    copy_o(n_heads - 1, bank).start()
    copy_o(n_heads - 2, 1 - bank).wait()
    copy_o(n_heads - 1, bank).wait()


def _attention(q, k, v, t, interpret=False):
    batch, heads, seq, dim = q.shape
    n_heads = batch * heads
    assert seq % BQ == 0 and n_heads >= 4 and n_heads % 2 == 0 and dim <= BK and seq // BQ > max(TAIL_QK, TAIL_PV)

    def to_head_major(x):
        return jnp.swapaxes(x, 2, 3).reshape(n_heads, dim, seq)

    in_hbm = pl.BlockSpec(memory_space=pl.ANY)
    out = pl.pallas_call(
        functools.partial(_attention_kernel, n_heads=n_heads, heads_per_batch=heads, seq=seq, dim=dim),
        in_specs=[in_hbm] * 4,
        out_specs=in_hbm,
        out_shape=jax.ShapeDtypeStruct((n_heads, dim, seq), q.dtype),
        scratch_shapes=(
            [pltpu.VMEM((2, 3, dim, seq), q.dtype), pltpu.VMEM((2, 2, dim, seq), q.dtype),
             pltpu.VMEM((2, dim, seq), q.dtype)]
            + [pltpu.VMEM((seq, dim), jnp.bfloat16)] * 2
            + [pltpu.VMEM((dim, seq), jnp.bfloat16)] * 2
            + [pltpu.VMEM((seq, seq), jnp.float32)] * 2
            + [pltpu.VMEM((1, seq), jnp.float32)] * 2
            + [pltpu.SemaphoreType.DMA((2,)), pltpu.SemaphoreType.DMA((2, 2)), pltpu.SemaphoreType.DMA((2,)),
               pltpu.VMEM((1, heads), t.dtype),
               pltpu.VMEM((1, heads), jnp.float32),
               pltpu.SMEM((1, heads), jnp.float32),
               pltpu.SemaphoreType.DMA((2,))]
        ),
        compiler_params=pltpu.CompilerParams(
            vmem_limit_bytes=100 * 1024 * 1024,
            disable_bounds_checks=True,
        ),
        interpret=interpret,
    )(t.reshape(1, heads), to_head_major(q), to_head_major(k), to_head_major(v))
    return jnp.swapaxes(out.reshape(batch, heads, dim, seq), 2, 3)


@jax.jit
def pallas_standalone__qk_norm__prompt_kernel(
    q: jax.Array,
    k: jax.Array,
    v: jax.Array,
    t: jax.Array,
):
    return _attention(q, k, v, t)
```
